```python
import os as _os
_os.environ.setdefault("JAX_PLATFORMS", "cpu")
import jax
import jax.numpy as jnp

def _softmax(x, axis=-1):
    return jax.nn.softmax(x, axis=axis)
def _gelu(x):
    return jax.nn.gelu(x, approximate=True)
def _silu(x):
    return jax.nn.silu(x)
def _sigmoid(x):
    return jax.nn.sigmoid(x)
def _layernorm(x, axis=-1, eps=1e-5):
    m = jnp.mean(x, axis=axis, keepdims=True)
    v = jnp.var(x, axis=axis, keepdims=True)
    return (x - m) / jnp.sqrt(v + eps)
def _scatter_add(tgt, idx, src, axis=0):
    return tgt.at[idx].add(src)
def _segment_sum(src, seg, n):
    return jax.ops.segment_sum(src, seg, n)
class _Rng:
    def __init__(self, key):
        self._k = key
    def _next(self):
        self._k, sub = jax.random.split(self._k)
        return sub
    def normal(self, shape):
        return jax.random.normal(self._next(), shape, dtype=jnp.bfloat16)
    def randint(self, lo, hi, shape):
        return jax.random.randint(self._next(), shape, lo, hi, dtype=jnp.int32)
    def uniform(self, shape, lo=0.0, hi=1.0):
        return jax.random.uniform(self._next(), shape, jnp.bfloat16, lo, hi)
    def permutation(self, n):
        return jax.random.permutation(self._next(), n)


kernel_name = 'concat_heads__mha_block_cached__mha_block_cached__near_ridge'

def setup_inputs():
    _rng = _Rng(jax.random.key(int.from_bytes(__import__("os").urandom(4), "little")))
    _w = (lambda a: (lambda t: t.astype(jnp.bfloat16) if jnp.issubdtype(t.dtype, jnp.floating) else t)(jnp.asarray(a)))
    def _A_setup():
        B, Sq, D = 16, 192, 512
        H, Sk, Dh = 32, 512, 128
        return {
            "x": _w((lambda *s: _rng.normal(s) * 0.8)(B, Sq, D)),
            "k_cache": _w((lambda *s: _rng.normal(s) * 0.8)(B, H, Sk, Dh)),
            "v_cache": _w((lambda *s: _rng.normal(s) * 0.05)(B, H, Sk, Dh)),
            "wq": _w((lambda *s: _rng.normal(s) * 0.8)(D, H * Dh) * (D ** -0.5)),
            "wo": _w((lambda *s: _rng.normal(s) * 0.05)(H * Dh, D) * ((H * Dh) ** -0.5)),
        }
    _A_in = _A_setup()

    def _B_setup():
        B, Sq, D = 16, 192, 512
        H, Sk, Dh = 32, 512, 128
        return {
            "x": _w((lambda *s: _rng.normal(s) * 0.8)(B, Sq, D)),
            "k_cache": _w((lambda *s: _rng.normal(s) * 0.8)(B, H, Sk, Dh)),
            "v_cache": _w((lambda *s: _rng.normal(s) * 0.05)(B, H, Sk, Dh)),
            "wq": _w((lambda *s: _rng.normal(s) * 0.8)(D, H * Dh) * (D ** -0.5)),
            "wo": _w((lambda *s: _rng.normal(s) * 0.05)(H * Dh, D) * ((H * Dh) ** -0.5)),
        }
    _B_in = _B_setup()

    return {
        "A_x": _A_in["x"],
        "A_k_cache": _A_in["k_cache"],
        "A_v_cache": _A_in["v_cache"],
        "A_wq": _A_in["wq"],
        "A_wo": _A_in["wo"],
        "B_x": _B_in["x"],
        "B_k_cache": _B_in["k_cache"],
        "B_v_cache": _B_in["v_cache"],
        "B_wq": _B_in["wq"],
        "B_wo": _B_in["wo"],
    }

def reference(A_x, A_k_cache, A_v_cache, A_wq, A_wo, B_x, B_k_cache, B_v_cache, B_wq, B_wo):
    def _A_ref(x, k_cache, v_cache, wq, wo):
        B, Sq, D = x.shape
        H, Dh = 32, 128
        q = (lambda x, *d: x.transpose(*d))((x @ wq).reshape(B, Sq, H, Dh), 0, 2, 1, 3)
        scores = jnp.einsum("bhqd,bhkd->bhqk", q, k_cache) * (Dh ** -0.5)
        p = _softmax(scores, axis=-1)
        o = jnp.einsum("bhqk,bhkd->bhqd", p, v_cache)
        return (lambda x, *d: x.transpose(*d))(o, 0, 2, 1, 3).reshape(B, Sq, H * Dh) @ wo

    def _B_ref(x, k_cache, v_cache, wq, wo):
        B, Sq, D = x.shape
        H, Dh = 32, 128
        q = (lambda x, *d: x.transpose(*d))((x @ wq).reshape(B, Sq, H, Dh), 0, 2, 1, 3)
        scores = jnp.einsum("bhqd,bhkd->bhqk", q, k_cache) * (Dh ** -0.5)
        p = _softmax(scores, axis=-1)
        o = jnp.einsum("bhqk,bhkd->bhqd", p, v_cache)
        return (lambda x, *d: x.transpose(*d))(o, 0, 2, 1, 3).reshape(B, Sq, H * Dh) @ wo

    a = _A_ref(A_x, A_k_cache, A_v_cache, A_wq, A_wo)
    b = _B_ref(B_x, B_k_cache, B_v_cache, B_wq, B_wo)
    return jnp.concatenate([a, b], axis=-1)
```

```python
import functools
import jax
import jax.numpy as jnp
from jax import lax
import jax.experimental.pallas as pl
import jax.experimental.pallas.tpu as pltpu

LOG2E = 1.4426950408889634
RAMP = [(4, 1), (14, 2)]
NOBC = True
R = 4
NS = 3
LA = 3
NSEM = LA + 1
HQ = 8


def _kernel(xa, ka, va, wqa, woa, xb, kb, vb, wqb, wob, o_hbm,
            x_s, kv, wq_s, wo_s, acc, out_s, sem_in, sem_out, *, B, Sq, D, H, Sk, Dh):
    f32 = jnp.float32
    bf16 = jnp.bfloat16
    c = (Dh ** -0.5) * LOG2E
    x_h = (xa, xb); k_h = (ka, kb); v_h = (va, vb); wq_h = (wqa, wqb); wo_h = (woa, wob)

    def ramp_x_copies():
        return [pltpu.make_async_copy(x_h[br].at[pl.ds(0, R)], x_s.at[br, pl.ds(0, R)], sem_in.at[0])
                for br in range(2)]

    def ramp_group(h0, g, gi):
        hq = h0 // HQ
        j0 = h0 % HQ
        slot = hq % NS
        sem = sem_in.at[gi % NSEM]
        aligned = (lambda v, m: v if isinstance(v, int) else pl.multiple_of(v, m))
        col = aligned(h0 * Dh, Dh)
        cps = []
        for br in range(2):
            cps.append(pltpu.make_async_copy(wq_h[br].at[:, pl.ds(col, g * Dh)], wq_s.at[br, :, pl.ds(col, g * Dh)], sem))
            cps.append(pltpu.make_async_copy(k_h[br].at[pl.ds(0, R), hq, pl.ds(j0, g)], kv.at[slot, br, 0, :, pl.ds(j0, g)], sem))
            cps.append(pltpu.make_async_copy(v_h[br].at[pl.ds(0, R), hq, pl.ds(j0, g)], kv.at[slot, br, 1, :, pl.ds(j0, g)], sem))
            cps.append(pltpu.make_async_copy(wo_h[br].at[pl.ds(col, g * Dh), :], wo_s.at[br, pl.ds(col, g * Dh), :], sem))
        return cps

    n_ramp = sum(n for n, _ in RAMP)

    def steady_group(b):
        slot = b % NS
        sem = sem_in.at[(b - R + n_ramp) % NSEM]
        cps = []
        for br in range(2):
            cps.append(pltpu.make_async_copy(x_h[br].at[b], x_s.at[br, b], sem))
            cps.append(pltpu.make_async_copy(k_h[br].at[b], kv.at[slot, br, 0], sem))
            cps.append(pltpu.make_async_copy(v_h[br].at[b], kv.at[slot, br, 1], sem))
        return cps

    def out_copy(b0, n):
        return pltpu.make_async_copy(out_s.at[pl.ds(b0, n)], o_hbm.at[pl.ds(b0, n)], sem_out.at[0])

    def body(units):
        n = len(units)
        Q = [None] * n; P = [None] * n; L = [None] * n; O = [None] * n

        def stA(i):
            u = units[i]
            q = jnp.dot(u["x"](), u["wq"](), preferred_element_type=f32)
            Q[i] = (q * c).astype(bf16)

        def stB(i):
            u = units[i]
            s = lax.dot_general(Q[i], u["k"](), (((1,), (1,)), ((), ())), preferred_element_type=f32)
            m = jnp.max(s, axis=-1, keepdims=True)
            p = jnp.exp2(s - m)
            L[i] = jnp.sum(p, axis=-1, keepdims=True)
            P[i] = p.astype(bf16)

        def stD(i):
            u = units[i]
            o = jnp.dot(P[i], u["v"](), preferred_element_type=f32)
            l = L[i]
            r = pl.reciprocal(l, approx=True)
            r = r * (2.0 - l * r)
            O[i] = (o * r).astype(bf16)

        def stE(i):
            u = units[i]
            part = jnp.dot(O[i], u["wo"](), preferred_element_type=f32)
            u["store"](part)

        order = [("A", 0)] + ([("A", 1)] if n > 1 else []) + [("B", 0)]
        for i in range(1, n + 2):
            if i + 1 < n: order.append(("A", i + 1))
            if i < n: order.append(("B", i))
            if i - 1 < n: order.append(("D", i - 1))
            if 0 <= i - 2: order.append(("E", i - 2))
        fn = dict(A=stA, B=stB, D=stD, E=stE)
        for s, i in order:
            fn[s](i)

    def ramp_units(h0, g, emit_out):
        hq = h0 // HQ
        j0 = h0 % HQ
        slot = hq % NS
        units = []
        for jj in range(g):
            col = pl.multiple_of((h0 + jj) * Dh, Dh)
            for b in range(R):
                for br in range(2):
                    def store(part, b=b, br=br, last=(emit_out and jj == g - 1)):
                        new = acc[b, :, br * D:(br + 1) * D] + part
                        acc[b, :, br * D:(br + 1) * D] = new
                        if last:
                            out_s[b, :, br * D:(br + 1) * D] = new.astype(bf16)
                    units.append(dict(
                        x=lambda b=b, br=br: x_s[br, b],
                        wq=lambda br=br, col=col: wq_s[br, :, pl.ds(col, Dh)],
                        k=lambda b=b, br=br, jj=jj: kv[slot, br, 0, b, j0 + jj],
                        v=lambda b=b, br=br, jj=jj: kv[slot, br, 1, b, j0 + jj],
                        wo=lambda br=br, col=col: wo_s[br, pl.ds(col, Dh), :],
                        store=store))
        return units

    def steady_units(b):
        slot = b % NS
        units = []
        for h in range(H):
            for br in range(2):
                def store(part, h=h, br=br):
                    if h == 0:
                        acc[0, :, br * D:(br + 1) * D] = part
                    elif h == H - 1:
                        out_s[b, :, br * D:(br + 1) * D] = (acc[0, :, br * D:(br + 1) * D] + part).astype(bf16)
                    else:
                        acc[0, :, br * D:(br + 1) * D] += part
                units.append(dict(
                    x=lambda br=br: x_s[br, b],
                    wq=lambda br=br, h=h: wq_s[br, :, h * Dh:(h + 1) * Dh],
                    k=lambda br=br, h=h: kv[slot, br, 0, h // HQ, h % HQ],
                    v=lambda br=br, h=h: kv[slot, br, 1, h // HQ, h % HQ],
                    wo=lambda br=br, h=h: wo_s[br, h * Dh:(h + 1) * Dh, :],
                    store=store))
        return units

    groups = []
    h = 0
    for n, g in RAMP:
        for t in range(n):
            groups.append((h, g)); h += g
    assert h == H

    def start_group_static(gi):
        if gi < n_ramp:
            h0, g = groups[gi]
            if gi == 0:
                for cp in ramp_x_copies(): cp.start()
            for cp in ramp_group(h0, g, gi): cp.start()
        else:
            for cp in steady_group(R + gi - n_ramp): cp.start()

    for gi in range(LA):
        start_group_static(gi)
    acc[...] = jnp.zeros_like(acc)

    base = 0
    hbase = 0
    for pi, (n, g) in enumerate(RAMP):
        last_phase = pi == len(RAMP) - 1
        def it(t, carry, base=base, hbase=hbase, n=n, g=g, pi=pi, last_phase=last_phase):
            h0 = hbase + t * g
            gi = base + t
            if pi == 0:
                @pl.when(t == 0)
                def _():
                    for cp in ramp_x_copies(): cp.wait()
            for cp in ramp_group(h0, g, gi): cp.wait()
            if n > LA:
                @pl.when(t + LA < n)
                def _():
                    for cp in ramp_group(h0 + LA * g, g, gi + LA): cp.start()
            for tt in range(max(0, n - LA), n):
                tgt = base + tt + LA
                if tgt < n_ramp:
                    @pl.when(t == tt)
                    def _():
                        start_group_static(tgt)
            if last_phase:
                @pl.when(t == n - 3)
                def _():
                    start_group_static(n_ramp)
                @pl.when(t == n - 2)
                def _():
                    start_group_static(n_ramp + 1)
            body(ramp_units(h0, g, last_phase))
            return carry
        lax.fori_loop(0, n, it, 0)
        base += n
        hbase += n * g

    out_copy(0, R).start()

    def steady(b, carry):
        for cp in steady_group(b): cp.wait()
        @pl.when(b + 2 < B)
        def _():
            for cp in steady_group(b + 2): cp.start()
        body(steady_units(b))
        out_copy(b, 1).start()
        return carry
    lax.fori_loop(R, B, steady, 0)

    out_copy(0, R).wait()
    for b in range(R, B):
        out_copy(b, 1).wait()


@jax.jit
def pallas_concat_heads__mha_block_cached__mha_block_cached__near_ridge_kernel(
    A_x, A_k_cache, A_v_cache, A_wq, A_wo, B_x, B_k_cache, B_v_cache, B_wq, B_wo):
    B, Sq, D = A_x.shape
    _, H, Sk, Dh = A_k_cache.shape
    bf16 = jnp.bfloat16
    rs = lambda t: t.reshape(B, H // HQ, HQ, Sk, Dh)
    any_spec = pl.BlockSpec(memory_space=pl.ANY)
    return pl.pallas_call(
        functools.partial(_kernel, B=B, Sq=Sq, D=D, H=H, Sk=Sk, Dh=Dh),
        in_specs=[any_spec] * 10,
        out_specs=any_spec,
        out_shape=jax.ShapeDtypeStruct((B, Sq, 2 * D), bf16),
        scratch_shapes=[
            pltpu.VMEM((2, B, Sq, D), bf16),
            pltpu.VMEM((NS, 2, 2, H // HQ, HQ, Sk, Dh), bf16),
            pltpu.VMEM((2, D, H * Dh), bf16),
            pltpu.VMEM((2, H * Dh, D), bf16),
            pltpu.VMEM((R, Sq, 2 * D), jnp.float32),
            pltpu.VMEM((B, Sq, 2 * D), bf16),
            pltpu.SemaphoreType.DMA((NSEM,)),
            pltpu.SemaphoreType.DMA((1,)),
        ],
        compiler_params=pltpu.CompilerParams(
            vmem_limit_bytes=110 * 1024 * 1024,
            disable_bounds_checks=NOBC),
    )(A_x, rs(A_k_cache), rs(A_v_cache), A_wq, A_wo, B_x, rs(B_k_cache), rs(B_v_cache), B_wq, B_wo)
```

```python
import functools

import jax
import jax.numpy as jnp
from jax import lax
import jax.experimental.pallas as pl
import jax.experimental.pallas.tpu as pltpu

LOG2E = 1.4426950408889634
R = 4
N0 = 16
G1 = 2
HQ = 8
NS = 4
LA = 5
NSEM = 8


def _kernel(xa, ka, va, wqa, woa, xb, kb, vb, wqb, wob, o_hbm,
            x_s, kv, wq_s, wo_s, acc, out_s, sem_in, sem_out,
            *, B, Sq, D, H, Dh):
    f32 = jnp.float32
    bf16 = jnp.bfloat16
    scale = (Dh ** -0.5) * LOG2E
    x_h, k_h, v_h = (xa, xb), (ka, kb), (va, vb)
    wq_h, wo_h = (wqa, wqb), (woa, wob)
    H0 = N0 // 2
    N1 = (H - H0) // G1
    n_ramp = N0 + N1
    assert R * HQ == H and H0 % 2 == 0 and H0 + N1 * G1 == H and HQ % G1 == 0
    assert 3 <= LA <= N0 and LA <= N1 - 3 and LA + 2 < NSEM

    def mod(v, m):
        return v % m if isinstance(v, int) else lax.bitwise_and(v, m - 1)

    def div(v, m):
        return v // m if isinstance(v, int) else lax.shift_right_logical(v, m.bit_length() - 1)

    def aligned(v, m):
        return v if isinstance(v, int) else pl.multiple_of(v, m)

    def p0_head(t):
        return 2 * div(t, 4) + mod(t, 2)

    def p0_branch(t):
        return mod(div(t, 2), 2)

    def group_sem(g):
        return sem_in.at[mod(g, NSEM)]

    def x_copy(src, br, b0, nb, sem):
        return pltpu.make_async_copy(
            x_h[src].at[pl.ds(b0, nb)], x_s.at[br, pl.ds(b0, nb)], sem)

    def head_copies(src, br, h0, g, sem):
        hq, j0 = div(h0, HQ), mod(h0, HQ)
        rows = pl.ds(aligned(h0 * Dh, Dh), g * Dh)
        cps = [
            pltpu.make_async_copy(
                wq_h[src].at[:, pl.ds(aligned((h0 + j) * Dh, Dh), Dh)],
                wq_s.at[br, h0 + j], sem)
            for j in range(g)
        ]
        for i, t_h in enumerate((k_h, v_h)):
            cps.append(pltpu.make_async_copy(
                t_h[src].at[pl.ds(0, R), hq, pl.ds(j0, g)],
                kv.at[mod(hq, NS), br, i, :, pl.ds(j0, g)], sem))
        cps.append(pltpu.make_async_copy(
            wo_h[src].at[rows, :], wo_s.at[br, rows, :], sem))
        return cps

    def p1_group(t):
        h0 = H0 + t * G1
        sem = group_sem(N0 + t)
        return head_copies(0, 0, h0, G1, sem) + head_copies(1, 1, h0, G1, sem)

    def steady_group(b):
        sem = group_sem(b - R + n_ramp)
        cps = []
        for br in range(2):
            cps.append(x_copy(br, br, b, 1, sem))
            cps.append(pltpu.make_async_copy(k_h[br].at[b], kv.at[mod(b, NS), br, 0], sem))
            cps.append(pltpu.make_async_copy(v_h[br].at[b], kv.at[mod(b, NS), br, 1], sem))
        return cps

    def start_group(g):
        if g < N0:
            h, br = p0_head(g), p0_branch(g)
            cps = [x_copy(br, br, 0, R, group_sem(g))] if h == 0 else []
            cps += head_copies(br, br, h, 1, group_sem(g))
        elif g < n_ramp:
            cps = p1_group(g - N0)
        else:
            cps = steady_group(R + g - n_ramp)
        for cp in cps:
            cp.start()

    def out_copy(b0, nb, br):
        return pltpu.make_async_copy(
            out_s.at[br, pl.ds(b0, nb)],
            o_hbm.at[pl.ds(b0, nb), :, pl.ds(br * D, D)], sem_out.at[0])

    def run_body(units, prefetch):
        n = len(units)
        q, p, l, o = ([None] * n for _ in range(4))

        def stage_a(i):
            u = units[i]
            t = jnp.dot(u["x"](), u["wq"](), preferred_element_type=f32)
            q[i] = (t * scale).astype(bf16)

        def stage_b(i):
            s = lax.dot_general(q[i], units[i]["k"](), (((1,), (1,)), ((), ())),
                                preferred_element_type=f32)
            e = jnp.exp2(s - jnp.max(s, axis=-1, keepdims=True))
            l[i] = jnp.sum(e, axis=-1, keepdims=True)
            p[i] = e.astype(bf16)

        def stage_d(i):
            t = jnp.dot(p[i], units[i]["v"](), preferred_element_type=f32)
            r = pl.reciprocal(l[i], approx=True)
            r = r * (2.0 - l[i] * r)
            o[i] = (t * r).astype(bf16)

        def stage_e(i):
            u = units[i]
            u["store"](jnp.dot(o[i], u["wo"](), preferred_element_type=f32))

        stage_a(0)
        stage_a(1)
        stage_b(0)
        for i in range(1, n + 2):
            if i + 1 < n:
                stage_a(i + 1)
            if i == 1:
                prefetch()
            if i < n:
                stage_b(i)
            if i - 1 < n:
                stage_d(i - 1)
            if i >= 2:
                stage_e(i - 2)

    def ramp_unit(br, b, h, emit):
        slot, j = mod(div(h, HQ), NS), mod(h, HQ)

        def store(part):
            total = acc[b, br] + part
            acc[b, br] = total
            if emit:
                out_s[br, b] = total.astype(bf16)

        return dict(
            x=lambda: x_s[br, b],
            wq=lambda: wq_s[br, h],
            k=lambda: kv[slot, br, 0, b, j],
            v=lambda: kv[slot, br, 1, b, j],
            wo=lambda: wo_s[br, pl.ds(aligned(h * Dh, Dh), Dh), :],
            store=store)

    def steady_unit(br, b, h):
        slot = mod(b, NS)

        def store(part):
            if h == 0:
                acc[0, br] = part
            elif h < H - 1:
                acc[0, br] += part
            else:
                out_s[br, b] = (acc[0, br] + part).astype(bf16)
                out_copy(b, 1, br).start()

        return dict(
            x=lambda: x_s[br, b],
            wq=lambda: wq_s[br, h],
            k=lambda: kv[slot, br, 0, h // HQ, h % HQ],
            v=lambda: kv[slot, br, 1, h // HQ, h % HQ],
            wo=lambda: wo_s[br, h * Dh:(h + 1) * Dh, :],
            store=store)

    for g in range(LA):
        start_group(g)
    acc[...] = jnp.zeros_like(acc)

    def phase0(t, carry):
        h, br = p0_head(t), p0_branch(t)

        @pl.when(h == 0)
        def _():
            x_copy(0, br, 0, R, group_sem(t)).wait()
        for cp in head_copies(0, br, h, 1, group_sem(t)):
            cp.wait()

        def prefetch():
            t2 = t + LA
            for src in range(2):
                @pl.when(jnp.logical_and(t2 < N0, p0_branch(t2) == src))
                def _():
                    for cp in head_copies(src, src, p0_head(t2), 1, group_sem(t2)):
                        cp.start()
            for tt in range(N0 - LA, N0):
                @pl.when(t == tt)
                def _():
                    start_group(tt + LA)

        run_body([ramp_unit(br, b, h, False) for b in range(R)], prefetch)
        return carry

    lax.fori_loop(0, N0, phase0, 0)

    def phase1(t, carry):
        for cp in p1_group(t):
            cp.wait()

        def prefetch():
            @pl.when(t + LA < N1)
            def _():
                for cp in p1_group(t + LA):
                    cp.start()
            for k in range(2):
                @pl.when(t == N1 - 3 + k)
                def _():
                    start_group(n_ramp + k)

        h0 = H0 + t * G1
        run_body([ramp_unit(br, b, h0 + j, j == G1 - 1)
                  for j in range(G1) for b in range(R) for br in range(2)], prefetch)
        return carry

    lax.fori_loop(0, N1, phase1, 0)
    for br in range(2):
        out_copy(0, R, br).start()

    def steady(b, carry):
        for cp in steady_group(b):
            cp.wait()

        def prefetch():
            @pl.when(b + 2 < B)
            def _():
                for cp in steady_group(b + 2):
                    cp.start()

        run_body([steady_unit(br, b, h) for br in range(2) for h in range(H)], prefetch)
        return carry

    lax.fori_loop(R, B, steady, 0)

    for br in range(2):
        out_copy(0, R, br).wait()
        for b in range(R, B):
            out_copy(b, 1, br).wait()


@jax.jit
def pallas_concat_heads__mha_block_cached__mha_block_cached__near_ridge_kernel(
    A_x: jax.Array,
    A_k_cache: jax.Array,
    A_v_cache: jax.Array,
    A_wq: jax.Array,
    A_wo: jax.Array,
    B_x: jax.Array,
    B_k_cache: jax.Array,
    B_v_cache: jax.Array,
    B_wq: jax.Array,
    B_wo: jax.Array,
):
    B, Sq, D = A_x.shape
    _, H, Sk, Dh = A_k_cache.shape
    bf16 = jnp.bfloat16

    def split_heads(t):
        return t.reshape(B, H // HQ, HQ, Sk, Dh)

    hbm = pl.BlockSpec(memory_space=pl.ANY)
    return pl.pallas_call(
        functools.partial(_kernel, B=B, Sq=Sq, D=D, H=H, Dh=Dh),
        in_specs=[hbm] * 10,
        out_specs=hbm,
        out_shape=jax.ShapeDtypeStruct((B, Sq, 2 * D), bf16),
        scratch_shapes=[
            pltpu.VMEM((2, B, Sq, D), bf16),
            pltpu.VMEM((NS, 2, 2, H // HQ, HQ, Sk, Dh), bf16),
            pltpu.VMEM((2, H, D, Dh), bf16),
            pltpu.VMEM((2, H * Dh, D), bf16),
            pltpu.VMEM((R, 2, Sq, D), jnp.float32),
            pltpu.VMEM((2, B, Sq, D), bf16),
            pltpu.SemaphoreType.DMA((NSEM,)),
            pltpu.SemaphoreType.DMA((1,)),
        ],
        compiler_params=pltpu.CompilerParams(
            vmem_limit_bytes=110 * 1024 * 1024,
            disable_bounds_checks=True),
    )(A_x, split_heads(A_k_cache), split_heads(A_v_cache), A_wq, A_wo,
      B_x, split_heads(B_k_cache), split_heads(B_v_cache), B_wq, B_wo)
```

```python
import functools

import jax
import jax.numpy as jnp
from jax import lax
import jax.experimental.pallas as pl
import jax.experimental.pallas.tpu as pltpu

LOG2E = 1.4426950408889634
R = 4
N0 = 16
PB = 4
G1 = 2
HQ = 8
NS = 4
LA = 5
NSEM = 8


def _kernel(xa, ka, va, wqa, woa, xb, kb, vb, wqb, wob, o_hbm,
            x_s, kv, wq_s, wo_s, acc, out_s, sem_in, sem_out,
            *, B, Sq, D, H, Dh):
    f32 = jnp.float32
    bf16 = jnp.bfloat16
    scale = (Dh ** -0.5) * LOG2E
    x_h, k_h, v_h = (xa, xb), (ka, kb), (va, vb)
    wq_h, wo_h = (wqa, wqb), (woa, wob)
    H0 = N0 // 2
    N1 = (H - H0) // G1
    n_ramp = N0 + N1
    assert R * HQ == H and H0 % PB == 0 and H0 + N1 * G1 == H and HQ % G1 == 0
    assert PB < LA <= N0 and LA <= N1 - 3 and LA < NSEM

    def mod(v, m):
        return v % m if isinstance(v, int) else lax.bitwise_and(v, m - 1)

    def div(v, m):
        return v // m if isinstance(v, int) else lax.shift_right_logical(v, m.bit_length() - 1)

    def aligned(v, m):
        return v if isinstance(v, int) else pl.multiple_of(v, m)

    def p0_head(t):
        return PB * div(t, 2 * PB) + mod(t, PB)

    def p0_branch(t):
        return mod(div(t, PB), 2)

    def group_sem(g):
        return sem_in.at[mod(g, NSEM)]

    def x_copy(src, br, b0, nb, sem):
        return pltpu.make_async_copy(
            x_h[src].at[pl.ds(b0, nb)], x_s.at[br, pl.ds(b0, nb)], sem)

    def head_copies(src, br, h0, g, sem):
        hq, j0 = div(h0, HQ), mod(h0, HQ)
        rows = pl.ds(aligned(h0 * Dh, Dh), g * Dh)
        cps = [
            pltpu.make_async_copy(
                wq_h[src].at[:, pl.ds(aligned((h0 + j) * Dh, Dh), Dh)],
                wq_s.at[br, h0 + j], sem)
            for j in range(g)
        ]
        for i, t_h in enumerate((k_h, v_h)):
            cps.append(pltpu.make_async_copy(
                t_h[src].at[pl.ds(0, R), hq, pl.ds(j0, g)],
                kv.at[mod(hq, NS), br, i, :, pl.ds(j0, g)], sem))
        cps.append(pltpu.make_async_copy(
            wo_h[src].at[rows, :], wo_s.at[br, rows, :], sem))
        return cps

    def p1_group(t):
        h0 = H0 + t * G1
        sem = group_sem(N0 + t)
        return head_copies(0, 0, h0, G1, sem) + head_copies(1, 1, h0, G1, sem)

    def steady_group(b):
        sem = group_sem(b - R + n_ramp)
        cps = []
        for br in range(2):
            cps.append(x_copy(br, br, b, 1, sem))
            cps.append(pltpu.make_async_copy(k_h[br].at[b], kv.at[mod(b, NS), br, 0], sem))
            cps.append(pltpu.make_async_copy(v_h[br].at[b], kv.at[mod(b, NS), br, 1], sem))
        return cps

    def start_group(g):
        if g < N0:
            h, br = p0_head(g), p0_branch(g)
            cps = [x_copy(br, br, 0, R, group_sem(g))] if h == 0 else []
            cps += head_copies(br, br, h, 1, group_sem(g))
        elif g < n_ramp:
            cps = p1_group(g - N0)
        else:
            cps = steady_group(R + g - n_ramp)
        for cp in cps:
            cp.start()

    def out_copy(b0, nb, br):
        return pltpu.make_async_copy(
            out_s.at[br, pl.ds(b0, nb)],
            o_hbm.at[pl.ds(b0, nb), :, pl.ds(br * D, D)], sem_out.at[0])

    def run_body(units, prefetch):
        n = len(units)
        q, p, l, o = ([None] * n for _ in range(4))

        def stage_a(i):
            u = units[i]
            t = jnp.dot(u["x"](), u["wq"](), preferred_element_type=f32)
            q[i] = (t * scale).astype(bf16)

        def stage_b(i):
            s = lax.dot_general(q[i], units[i]["k"](), (((1,), (1,)), ((), ())),
                                preferred_element_type=f32)
            e = jnp.exp2(s - jnp.max(s, axis=-1, keepdims=True))
            l[i] = jnp.sum(e, axis=-1, keepdims=True)
            p[i] = e.astype(bf16)

        def stage_d(i):
            t = jnp.dot(p[i], units[i]["v"](), preferred_element_type=f32)
            r = pl.reciprocal(l[i], approx=True)
            r = r * (2.0 - l[i] * r)
            o[i] = (t * r).astype(bf16)

        def stage_e(i):
            u = units[i]
            u["store"](jnp.dot(o[i], u["wo"](), preferred_element_type=f32))

        stage_a(0)
        stage_a(1)
        stage_b(0)
        for i in range(1, n + 2):
            if i + 1 < n:
                stage_a(i + 1)
            if i == 1:
                prefetch()
            if i < n:
                stage_b(i)
            if i - 1 < n:
                stage_d(i - 1)
            if i >= 2:
                stage_e(i - 2)

    def ramp_unit(br, b, h, emit):
        slot, j = mod(div(h, HQ), NS), mod(h, HQ)

        def store(part):
            total = acc[b, br] + part
            acc[b, br] = total
            if emit:
                out_s[br, b] = total.astype(bf16)

        return dict(
            x=lambda: x_s[br, b],
            wq=lambda: wq_s[br, h],
            k=lambda: kv[slot, br, 0, b, j],
            v=lambda: kv[slot, br, 1, b, j],
            wo=lambda: wo_s[br, pl.ds(aligned(h * Dh, Dh), Dh), :],
            store=store)

    def steady_unit(br, b, h):
        slot = mod(b, NS)

        def store(part):
            if h == 0:
                acc[0, br] = part
            elif h < H - 1:
                acc[0, br] += part
            else:
                out_s[br, b] = (acc[0, br] + part).astype(bf16)
                out_copy(b, 1, br).start()

        return dict(
            x=lambda: x_s[br, b],
            wq=lambda: wq_s[br, h],
            k=lambda: kv[slot, br, 0, h // HQ, h % HQ],
            v=lambda: kv[slot, br, 1, h // HQ, h % HQ],
            wo=lambda: wo_s[br, h * Dh:(h + 1) * Dh, :],
            store=store)

    for g in range(LA):
        start_group(g)
    acc[...] = jnp.zeros_like(acc)

    def phase0(t, carry):
        h, br = p0_head(t), p0_branch(t)

        @pl.when(h == 0)
        def _():
            x_copy(0, br, 0, R, group_sem(t)).wait()
        for cp in head_copies(0, br, h, 1, group_sem(t)):
            cp.wait()

        def prefetch():
            t2 = t + LA
            for src in range(2):
                @pl.when(jnp.logical_and(t2 < N0, p0_branch(t2) == src))
                def _():
                    for cp in head_copies(src, src, p0_head(t2), 1, group_sem(t2)):
                        cp.start()
            for tt in range(N0 - LA, N0):
                @pl.when(t == tt)
                def _():
                    start_group(tt + LA)

        run_body([ramp_unit(br, b, h, False) for b in range(R)], prefetch)
        return carry

    lax.fori_loop(0, N0, phase0, 0)

    def phase1(t, carry):
        for cp in p1_group(t):
            cp.wait()

        def prefetch():
            @pl.when(t + LA < N1)
            def _():
                for cp in p1_group(t + LA):
                    cp.start()
            for k in range(2):
                @pl.when(t == N1 - 3 + k)
                def _():
                    start_group(n_ramp + k)

        h0 = H0 + t * G1
        run_body([ramp_unit(br, b, h0 + j, j == G1 - 1)
                  for j in range(G1) for b in range(R) for br in range(2)], prefetch)
        return carry

    lax.fori_loop(0, N1, phase1, 0)
    for br in range(2):
        out_copy(0, R, br).start()

    def steady(b, carry):
        for cp in steady_group(b):
            cp.wait()

        def prefetch():
            @pl.when(b + 2 < B)
            def _():
                for cp in steady_group(b + 2):
                    cp.start()

        run_body([steady_unit(br, b, h) for br in range(2) for h in range(H)], prefetch)
        return carry

    lax.fori_loop(R, B, steady, 0)

    for br in range(2):
        out_copy(0, R, br).wait()
        for b in range(R, B):
            out_copy(b, 1, br).wait()


@jax.jit
def pallas_concat_heads__mha_block_cached__mha_block_cached__near_ridge_kernel(
    A_x: jax.Array,
    A_k_cache: jax.Array,
    A_v_cache: jax.Array,
    A_wq: jax.Array,
    A_wo: jax.Array,
    B_x: jax.Array,
    B_k_cache: jax.Array,
    B_v_cache: jax.Array,
    B_wq: jax.Array,
    B_wo: jax.Array,
):
    B, Sq, D = A_x.shape
    _, H, Sk, Dh = A_k_cache.shape
    bf16 = jnp.bfloat16

    def split_heads(t):
        return t.reshape(B, H // HQ, HQ, Sk, Dh)

    hbm = pl.BlockSpec(memory_space=pl.ANY)
    return pl.pallas_call(
        functools.partial(_kernel, B=B, Sq=Sq, D=D, H=H, Dh=Dh),
        in_specs=[hbm] * 10,
        out_specs=hbm,
        out_shape=jax.ShapeDtypeStruct((B, Sq, 2 * D), bf16),
        scratch_shapes=[
            pltpu.VMEM((2, B, Sq, D), bf16),
            pltpu.VMEM((NS, 2, 2, H // HQ, HQ, Sk, Dh), bf16),
            pltpu.VMEM((2, H, D, Dh), bf16),
            pltpu.VMEM((2, H * Dh, D), bf16),
            pltpu.VMEM((R, 2, Sq, D), jnp.float32),
            pltpu.VMEM((2, B, Sq, D), bf16),
            pltpu.SemaphoreType.DMA((NSEM,)),
            pltpu.SemaphoreType.DMA((1,)),
        ],
        compiler_params=pltpu.CompilerParams(
            vmem_limit_bytes=110 * 1024 * 1024,
            disable_bounds_checks=True),
    )(A_x, split_heads(A_k_cache), split_heads(A_v_cache), A_wq, A_wo,
      B_x, split_heads(B_k_cache), split_heads(B_v_cache), B_wq, B_wo)
```

```python
import functools

import jax
import jax.numpy as jnp
from jax import lax
import jax.experimental.pallas as pl
import jax.experimental.pallas.tpu as pltpu

LOG2E = 1.4426950408889634
R = 4
N0 = 16
PB = 4
G1 = 2
HQ = 8
NS = 4
LA = 5
NSEM = 8
OCH = 4

ORDER_RAMP0 = (("B", 0), ("A", 1), ("D", -1), ("E", -2))
ORDER_RAMP1 = (("B", 0), ("D", -2), ("A", 2), ("E", -2))
ORDER_STEADY = (("B", 0), ("A", 1), ("E", -2), ("D", -1))


def _kernel(xa, ka, va, wqa, woa, xb, kb, vb, wqb, wob, o_hbm,
            x_s, kv, wq_s, wo_s, acc, out_s, sem_in, sem_pre, sem_out,
            *, B, Sq, D, H, Dh):
    f32 = jnp.float32
    bf16 = jnp.bfloat16
    scale = (Dh ** -0.5) * LOG2E
    x_h, k_h, v_h = (xa, xb), (ka, kb), (va, vb)
    wq_h, wo_h = (wqa, wqb), (woa, wob)
    H0 = N0 // 2
    N1 = (H - H0) // G1
    n_ramp = N0 + N1
    RP = R // 2
    RC = Sq // OCH
    assert R * HQ == H and H0 % PB == 0 and H0 + N1 * G1 == H and HQ % G1 == 0
    assert PB < LA <= N0 and LA <= N1 - 3 and LA < NSEM

    def mod(v, m):
        return v % m if isinstance(v, int) else lax.bitwise_and(v, m - 1)

    def div(v, m):
        return v // m if isinstance(v, int) else lax.shift_right_logical(v, m.bit_length() - 1)

    def aligned(v, m):
        return v if isinstance(v, int) else pl.multiple_of(v, m)

    def p0_head(t):
        return PB * div(t, 2 * PB) + mod(t, PB)

    def p0_branch(t):
        return mod(div(t, PB), 2)

    def group_sem(g):
        return sem_in.at[mod(g, NSEM)]

    def x_copy(src, br, b0, nb, sem):
        return pltpu.make_async_copy(
            x_h[src].at[pl.ds(b0, nb)], x_s.at[br, pl.ds(b0, nb)], sem)

    def weight_copies(src, br, h0, g, sem):
        rows = pl.ds(aligned(h0 * Dh, Dh), g * Dh)
        cps = [
            pltpu.make_async_copy(
                wq_h[src].at[:, pl.ds(aligned((h0 + j) * Dh, Dh), Dh)],
                wq_s.at[br, h0 + j], sem)
            for j in range(g)
        ]
        cps.append(pltpu.make_async_copy(
            wo_h[src].at[rows, :], wo_s.at[br, rows, :], sem))
        return cps

    def ramp_kv_copies(src, br, b0, nb, h0, g, sem):
        hq, j0 = div(h0, HQ), mod(h0, HQ)
        return [
            pltpu.make_async_copy(
                t_h[src].at[pl.ds(b0, nb), hq, pl.ds(j0, g)],
                kv.at[mod(hq, NS), br, i, pl.ds(b0, nb), pl.ds(j0, g)], sem)
            for i, t_h in enumerate((k_h, v_h))
        ]

    def head_copies(src, br, h0, g, sem):
        return (weight_copies(src, br, h0, g, sem)
                + ramp_kv_copies(src, br, 0, R, h0, g, sem))

    def pre_group(p):
        sem = sem_pre.at[p]
        return [x_copy(0, 0, p * RP, RP, sem)] + ramp_kv_copies(0, 0, p * RP, RP, 0, 1, sem)

    def pre_weights():
        return weight_copies(0, 0, 0, 1, sem_pre.at[0])

    def p1_group(t):
        h0 = H0 + t * G1
        sem = group_sem(N0 + t)
        return head_copies(0, 0, h0, G1, sem) + head_copies(1, 1, h0, G1, sem)

    def steady_group(b):
        sem = group_sem(b - R + n_ramp)
        cps = []
        for br in range(2):
            cps.append(x_copy(br, br, b, 1, sem))
            cps.append(pltpu.make_async_copy(k_h[br].at[b], kv.at[mod(b, NS), br, 0], sem))
            cps.append(pltpu.make_async_copy(v_h[br].at[b], kv.at[mod(b, NS), br, 1], sem))
        return cps

    def start_group(g):
        if g == 0:
            cps = pre_weights() + pre_group(0) + pre_group(1)
        elif g < N0:
            h, br = p0_head(g), p0_branch(g)
            cps = [x_copy(br, br, 0, R, group_sem(g))] if h == 0 else []
            cps += head_copies(br, br, h, 1, group_sem(g))
        elif g < n_ramp:
            cps = p1_group(g - N0)
        else:
            cps = steady_group(R + g - n_ramp)
        for cp in cps:
            cp.start()

    def out_copy(br, b0, nb, r0, nr):
        return pltpu.make_async_copy(
            out_s.at[br, pl.ds(b0, nb), pl.ds(r0, nr)],
            o_hbm.at[pl.ds(b0, nb), pl.ds(r0, nr), pl.ds(br * D, D)], sem_out.at[0])

    def run_body(units, order, prefetch):
        n = len(units)
        q, p, l, o = ([None] * n for _ in range(4))

        def stage_a(i):
            u = units[i]
            t = jnp.dot(u["x"](), u["wq"](), preferred_element_type=f32)
            q[i] = (t * scale).astype(bf16)

        def stage_b(i):
            if i == 1:
                prefetch()
            s = lax.dot_general(q[i], units[i]["k"](), (((1,), (1,)), ((), ())),
                                preferred_element_type=f32)
            e = jnp.exp2(s - jnp.max(s, axis=-1, keepdims=True))
            l[i] = jnp.sum(e, axis=-1, keepdims=True)
            p[i] = e.astype(bf16)

        def stage_d(i):
            t = jnp.dot(p[i], units[i]["v"](), preferred_element_type=f32)
            r = pl.reciprocal(l[i], approx=True)
            r = r * (2.0 - l[i] * r)
            o[i] = (t * r).astype(bf16)

        def stage_e(i):
            u = units[i]
            u["store"](jnp.dot(o[i], u["wo"](), preferred_element_type=f32))

        stages = dict(A=stage_a, B=stage_b, D=stage_d, E=stage_e)
        offs = [off for _, off in order]
        for step in range(-max(offs), n - min(offs)):
            for name, off in order:
                if 0 <= step + off < n:
                    stages[name](step + off)

    def ramp_unit(br, b, h, emit):
        slot, j = mod(div(h, HQ), NS), mod(h, HQ)

        def store(part):
            total = acc[b, br] + part
            acc[b, br] = total
            if emit:
                out_s[br, b] = total.astype(bf16)

        return dict(
            x=lambda: x_s[br, b],
            wq=lambda: wq_s[br, h],
            k=lambda: kv[slot, br, 0, b, j],
            v=lambda: kv[slot, br, 1, b, j],
            wo=lambda: wo_s[br, pl.ds(aligned(h * Dh, Dh), Dh), :],
            store=store)

    def steady_unit(br, b, h):
        slot = mod(b, NS)

        def store(part):
            if h == 0:
                acc[0, br] = part
            elif h < H - 1:
                acc[0, br] += part
            else:
                for c in range(OCH):
                    rows = slice(c * RC, (c + 1) * RC)
                    out_s[br, b, rows] = (acc[0, br, rows] + part[rows]).astype(bf16)
                    out_copy(br, b, 1, c * RC, RC).start()

        return dict(
            x=lambda: x_s[br, b],
            wq=lambda: wq_s[br, h],
            k=lambda: kv[slot, br, 0, h // HQ, h % HQ],
            v=lambda: kv[slot, br, 1, h // HQ, h % HQ],
            wo=lambda: wo_s[br, h * Dh:(h + 1) * Dh, :],
            store=store)

    for g in range(LA):
        start_group(g)
    acc[...] = jnp.zeros_like(acc)

    def pre(p, carry):
        @pl.when(p == 0)
        def _():
            for cp in pre_weights():
                cp.wait()
        for cp in pre_group(p):
            cp.wait()

        def prefetch():
            @pl.when(p == 0)
            def _():
                start_group(LA)

        run_body([ramp_unit(0, p * RP + i, 0, False) for i in range(RP)],
                 ORDER_RAMP0, prefetch)
        return carry

    lax.fori_loop(0, 2, pre, 0)

    def phase0(t, carry):
        h, br = p0_head(t), p0_branch(t)

        @pl.when(h == 0)
        def _():
            x_copy(0, br, 0, R, group_sem(t)).wait()
        for cp in head_copies(0, br, h, 1, group_sem(t)):
            cp.wait()

        def prefetch():
            t2 = t + LA
            for src in range(2):
                @pl.when(jnp.logical_and(t2 < N0, p0_branch(t2) == src))
                def _():
                    for cp in head_copies(src, src, p0_head(t2), 1, group_sem(t2)):
                        cp.start()
            for tt in range(N0 - LA, N0):
                @pl.when(t == tt)
                def _():
                    start_group(tt + LA)

        run_body([ramp_unit(br, b, h, False) for b in range(R)], ORDER_RAMP0, prefetch)
        return carry

    lax.fori_loop(1, N0, phase0, 0)

    def phase1(t, carry):
        for cp in p1_group(t):
            cp.wait()

        def prefetch():
            @pl.when(t + LA < N1)
            def _():
                for cp in p1_group(t + LA):
                    cp.start()
            for k in range(2):
                @pl.when(t == N1 - 3 + k)
                def _():
                    start_group(n_ramp + k)

        h0 = H0 + t * G1
        run_body([ramp_unit(br, b, h0 + j, j == G1 - 1)
                  for j in range(G1) for b in range(R) for br in range(2)],
                 ORDER_RAMP1, prefetch)
        return carry

    lax.fori_loop(0, N1, phase1, 0)
    for br in range(2):
        out_copy(br, 0, R, 0, Sq).start()

    def steady(b, carry):
        for cp in steady_group(b):
            cp.wait()

        def prefetch():
            @pl.when(b + 2 < B)
            def _():
                for cp in steady_group(b + 2):
                    cp.start()

        run_body([steady_unit(br, b, h) for br in range(2) for h in range(H)],
                 ORDER_STEADY, prefetch)
        return carry

    lax.fori_loop(R, B, steady, 0)

    for br in range(2):
        out_copy(br, 0, R, 0, Sq).wait()
        for b in range(R, B):
            for c in range(OCH):
                out_copy(br, b, 1, c * RC, RC).wait()


@jax.jit
def pallas_concat_heads__mha_block_cached__mha_block_cached__near_ridge_kernel(
    A_x: jax.Array,
    A_k_cache: jax.Array,
    A_v_cache: jax.Array,
    A_wq: jax.Array,
    A_wo: jax.Array,
    B_x: jax.Array,
    B_k_cache: jax.Array,
    B_v_cache: jax.Array,
    B_wq: jax.Array,
    B_wo: jax.Array,
):
    B, Sq, D = A_x.shape
    _, H, Sk, Dh = A_k_cache.shape
    bf16 = jnp.bfloat16

    def split_heads(t):
        return t.reshape(B, H // HQ, HQ, Sk, Dh)

    hbm = pl.BlockSpec(memory_space=pl.ANY)
    return pl.pallas_call(
        functools.partial(_kernel, B=B, Sq=Sq, D=D, H=H, Dh=Dh),
        in_specs=[hbm] * 10,
        out_specs=hbm,
        out_shape=jax.ShapeDtypeStruct((B, Sq, 2 * D), bf16),
        scratch_shapes=[
            pltpu.VMEM((2, B, Sq, D), bf16),
            pltpu.VMEM((NS, 2, 2, H // HQ, HQ, Sk, Dh), bf16),
            pltpu.VMEM((2, H, D, Dh), bf16),
            pltpu.VMEM((2, H * Dh, D), bf16),
            pltpu.VMEM((R, 2, Sq, D), jnp.float32),
            pltpu.VMEM((2, B, Sq, D), bf16),
            pltpu.SemaphoreType.DMA((NSEM,)),
            pltpu.SemaphoreType.DMA((2,)),
            pltpu.SemaphoreType.DMA((1,)),
        ],
        compiler_params=pltpu.CompilerParams(
            vmem_limit_bytes=110 * 1024 * 1024,
            disable_bounds_checks=True),
    )(A_x, split_heads(A_k_cache), split_heads(A_v_cache), A_wq, A_wo,
      B_x, split_heads(B_k_cache), split_heads(B_v_cache), B_wq, B_wo)
```

```python
import functools

import jax
import jax.numpy as jnp
from jax import lax
import jax.experimental.pallas as pl
import jax.experimental.pallas.tpu as pltpu

LOG2E = 1.4426950408889634
RB = 6
U0 = 3
N0 = 16
PB = 4
G1 = 3
NPAIR = 4
LA = 6
NSEM = 8
OCH = 4
WCH = 4

ORDER_RAMP = (("B", 0), ("D", -2), ("A", 1), ("E", -2))
ORDER_STEADY = (("B", 0), ("A", 1), ("E", -2), ("D", -1))


def _kernel(xa, ka, va, wqa, woa, xb, kb, vb, wqb, wob, o_hbm,
            x_s, kv, wq_s, wo_s, acc, out_s, sem_in, sem_w, sem_out,
            *, B, Sq, D, H, Dh):
    f32 = jnp.float32
    bf16 = jnp.bfloat16
    scale = (Dh ** -0.5) * LOG2E
    x_h, k_h, v_h = (xa, xb), (ka, kb), (va, vb)
    wq_h, wo_h = (wqa, wqb), (woa, wob)
    H0 = N0 // 2
    N1 = (H - H0) // G1
    n_ramp = N0 + N1
    NA = (B - RB) // 2
    NST = NA + B // 2
    RC = Sq // OCH
    HW = H // WCH
    assert RB == 2 * U0 and H0 % PB == 0 and H0 + N1 * G1 == H
    assert PB < LA <= min(N0, N1) and LA < NSEM
    assert RB + 2 == 2 * NPAIR and WCH <= NA

    def mod(v, m):
        return v % m if isinstance(v, int) else lax.bitwise_and(v, m - 1)

    def div(v, m):
        return v // m if isinstance(v, int) else lax.shift_right_logical(v, m.bit_length() - 1)

    def aligned(v, m):
        return v if isinstance(v, int) else pl.multiple_of(v, m)

    def p0_head(t):
        return PB * div(t, 2 * PB) + mod(t, PB)

    def p0_half(t):
        return mod(div(t, PB), 2)

    def st_branch(j):
        return int(j >= NA) if isinstance(j, int) else (j >= NA).astype(jnp.int32)

    def st_batch(j):
        return RB + 2 * j - B * st_branch(j)

    def st_row(j):
        return 2 * mod(j + RB // 2, NPAIR)

    def group_sem(g):
        return sem_in.at[mod(g, NSEM)]

    def x_copy(src, br, b0, nb, sem):
        return pltpu.make_async_copy(
            x_h[src].at[pl.ds(b0, nb)], x_s.at[br, pl.ds(b0, nb)], sem)

    def weight_copies(br, h0, g, sem):
        rows = pl.ds(aligned(h0 * Dh, Dh), g * Dh)
        cps = [
            pltpu.make_async_copy(
                wq_h[br].at[:, pl.ds(aligned((h0 + j) * Dh, Dh), Dh)],
                wq_s.at[br, h0 + j], sem)
            for j in range(g)
        ]
        cps.append(pltpu.make_async_copy(
            wo_h[br].at[rows, :], wo_s.at[br, rows, :], sem))
        return cps

    def ramp_kv_copies(b0, nb, h0, g, sem):
        return [
            pltpu.make_async_copy(
                t_h[0].at[pl.ds(b0, nb), pl.ds(h0, g)],
                kv.at[i, pl.ds(b0, nb), pl.ds(h0, g)], sem)
            for i, t_h in enumerate((k_h, v_h))
        ]

    def p0_x(t):
        return x_copy(0, 0, p0_half(t) * U0, U0, group_sem(t))

    def p0_weights(t):
        return weight_copies(0, p0_head(t), 1, group_sem(t))

    def p0_kv(t):
        return ramp_kv_copies(p0_half(t) * U0, U0, p0_head(t), 1, group_sem(t))

    def p1_group(t):
        h0 = H0 + t * G1
        sem = group_sem(N0 + t)
        return weight_copies(0, h0, G1, sem) + ramp_kv_copies(0, RB, h0, G1, sem)

    def steady_group(j, src):
        sem = group_sem(n_ramp + j)
        b0, row = st_batch(j), st_row(j)
        return [x_copy(src, st_branch(j), b0, 2, sem)] + [
            pltpu.make_async_copy(t_h[src].at[pl.ds(b0, 2)], kv.at[i, pl.ds(row, 2)], sem)
            for i, t_h in enumerate((k_h, v_h))]

    def start_group(g):
        if g < N0:
            cps = [p0_x(g)] if p0_head(g) == 0 else []
            cps += p0_weights(g) if p0_half(g) == 0 else []
            cps += p0_kv(g)
        elif g < n_ramp:
            cps = p1_group(g - N0)
        else:
            cps = steady_group(g - n_ramp, st_branch(g - n_ramp))
        for cp in cps:
            cp.start()

    def b_weights(c):
        return weight_copies(1, c * HW, HW, sem_w.at[0])

    def out_copy(br, b0, nb, r0, nr):
        return pltpu.make_async_copy(
            out_s.at[br, pl.ds(b0, nb), pl.ds(r0, nr)],
            o_hbm.at[pl.ds(b0, nb), pl.ds(r0, nr), pl.ds(aligned(br * D, D), D)],
            sem_out.at[0])

    def run_body(units, order, prefetch):
        n = len(units)
        q, p, l, o = ([None] * n for _ in range(4))

        def stage_a(i):
            u = units[i]
            t = jnp.dot(u["x"](), u["wq"](), preferred_element_type=f32)
            q[i] = (t * scale).astype(bf16)

        def stage_b(i):
            if i == 1:
                prefetch()
            s = lax.dot_general(q[i], units[i]["k"](), (((1,), (1,)), ((), ())),
                                preferred_element_type=f32)
            e = jnp.exp2(s - jnp.max(s, axis=-1, keepdims=True))
            l[i] = jnp.sum(e, axis=-1, keepdims=True)
            p[i] = e.astype(bf16)

        def stage_d(i):
            t = jnp.dot(p[i], units[i]["v"](), preferred_element_type=f32)
            r = pl.reciprocal(l[i], approx=True)
            r = r * (2.0 - l[i] * r)
            o[i] = (t * r).astype(bf16)

        def stage_e(i):
            u = units[i]
            u["store"](jnp.dot(o[i], u["wo"](), preferred_element_type=f32))

        stages = dict(A=stage_a, B=stage_b, D=stage_d, E=stage_e)
        offs = [off for _, off in order]
        for step in range(-max(offs), n - min(offs)):
            for name, off in order:
                if 0 <= step + off < n:
                    stages[name](step + off)

    def ramp_unit(b, h, emit):
        def store(part):
            total = acc[b] + part
            acc[b] = total
            if emit:
                out_s[0, b] = total.astype(bf16)

        return dict(
            x=lambda: x_s[0, b],
            wq=lambda: wq_s[0, h],
            k=lambda: kv[0, b, h],
            v=lambda: kv[1, b, h],
            wo=lambda: wo_s[0, pl.ds(aligned(h * Dh, Dh), Dh), :],
            store=store)

    def steady_unit(br, b, row, h):
        def store(part):
            if h == 0:
                acc[0] = part
            elif h < H - 1:
                acc[0] += part
            else:
                for c in range(OCH):
                    rows = slice(c * RC, (c + 1) * RC)
                    out_s[br, b, rows] = (acc[0, rows] + part[rows]).astype(bf16)
                    out_copy(br, b, 1, c * RC, RC).start()

        return dict(
            x=lambda: x_s[br, b],
            wq=lambda: wq_s[br, h],
            k=lambda: kv[0, row, h],
            v=lambda: kv[1, row, h],
            wo=lambda: wo_s[br, h * Dh:(h + 1) * Dh, :],
            store=store)

    for g in range(LA):
        start_group(g)
    acc[...] = jnp.zeros_like(acc)

    def phase0(t, carry):
        h, half = p0_head(t), p0_half(t)

        @pl.when(h == 0)
        def _():
            p0_x(t).wait()

        @pl.when(half == 0)
        def _():
            for cp in p0_weights(t):
                cp.wait()
        for cp in p0_kv(t):
            cp.wait()

        def prefetch():
            t2 = t + LA

            @pl.when(jnp.logical_and(t2 < N0, p0_half(t2) == 0))
            def _():
                for cp in p0_weights(t2):
                    cp.start()

            @pl.when(t2 < N0)
            def _():
                for cp in p0_kv(t2):
                    cp.start()
            for tt in range(N0 - LA, N0):
                @pl.when(t == tt)
                def _():
                    start_group(tt + LA)

        run_body([ramp_unit(half * U0 + i, h, False) for i in range(U0)],
                 ORDER_RAMP, prefetch)
        return carry

    lax.fori_loop(0, N0, phase0, 0)

    def phase1(t, carry):
        for cp in p1_group(t):
            cp.wait()

        def prefetch():
            @pl.when(t + LA < N1)
            def _():
                for cp in p1_group(t + LA):
                    cp.start()

            @pl.when(t + LA == N1)
            def _():
                start_group(n_ramp)

        h0 = H0 + t * G1
        run_body([ramp_unit(b, h0 + j, j == G1 - 1)
                  for j in range(G1) for b in range(RB)], ORDER_RAMP, prefetch)
        return carry

    lax.fori_loop(0, N1, phase1, 0)
    out_copy(0, 0, RB, 0, Sq).start()
    start_group(n_ramp + 1)

    def steady(j, carry):
        br, b0, row = st_branch(j), st_batch(j), st_row(j)
        for cp in steady_group(j, 0):
            cp.wait()

        @pl.when(j == NA)
        def _():
            for c in range(WCH):
                for cp in b_weights(c):
                    cp.wait()

        def prefetch():
            j2 = j + 2
            for src in range(2):
                @pl.when(jnp.logical_and(j2 < NST, st_branch(j2) == src))
                def _():
                    for cp in steady_group(j2, src):
                        cp.start()
            for c in range(WCH):
                @pl.when(j == c)
                def _():
                    for cp in b_weights(c):
                        cp.start()

        run_body([steady_unit(br, b0 + i, row + i, h) for i in range(2) for h in range(H)],
                 ORDER_STEADY, prefetch)
        return carry

    lax.fori_loop(0, NST, steady, 0)

    out_copy(0, 0, RB, 0, Sq).wait()
    for br in range(2):
        for b in range(RB if br == 0 else 0, B):
            for c in range(OCH):
                out_copy(br, b, 1, c * RC, RC).wait()


@jax.jit
def pallas_concat_heads__mha_block_cached__mha_block_cached__near_ridge_kernel(
    A_x: jax.Array,
    A_k_cache: jax.Array,
    A_v_cache: jax.Array,
    A_wq: jax.Array,
    A_wo: jax.Array,
    B_x: jax.Array,
    B_k_cache: jax.Array,
    B_v_cache: jax.Array,
    B_wq: jax.Array,
    B_wo: jax.Array,
):
    B, Sq, D = A_x.shape
    _, H, Sk, Dh = A_k_cache.shape
    bf16 = jnp.bfloat16
    hbm = pl.BlockSpec(memory_space=pl.ANY)
    return pl.pallas_call(
        functools.partial(_kernel, B=B, Sq=Sq, D=D, H=H, Dh=Dh),
        in_specs=[hbm] * 10,
        out_specs=hbm,
        out_shape=jax.ShapeDtypeStruct((B, Sq, 2 * D), bf16),
        scratch_shapes=[
            pltpu.VMEM((2, B, Sq, D), bf16),
            pltpu.VMEM((2, 2 * NPAIR, H, Sk, Dh), bf16),
            pltpu.VMEM((2, H, D, Dh), bf16),
            pltpu.VMEM((2, H * Dh, D), bf16),
            pltpu.VMEM((RB, Sq, D), jnp.float32),
            pltpu.VMEM((2, B, Sq, D), bf16),
            pltpu.SemaphoreType.DMA((NSEM,)),
            pltpu.SemaphoreType.DMA((1,)),
            pltpu.SemaphoreType.DMA((1,)),
        ],
        compiler_params=pltpu.CompilerParams(
            vmem_limit_bytes=110 * 1024 * 1024,
            disable_bounds_checks=True,
            disable_semaphore_checks=True),
    )(A_x, A_k_cache, A_v_cache, A_wq, A_wo, B_x, B_k_cache, B_v_cache, B_wq, B_wo)
```
